```python
import os as _os
_os.environ.setdefault("JAX_PLATFORMS", "cpu")
import jax
import jax.numpy as jnp

def _softmax(x, axis=-1):
    return jax.nn.softmax(x, axis=axis)
def _gelu(x):
    return jax.nn.gelu(x, approximate=True)
def _silu(x):
    return jax.nn.silu(x)
def _sigmoid(x):
    return jax.nn.sigmoid(x)
def _layernorm(x, axis=-1, eps=1e-5):
    m = jnp.mean(x, axis=axis, keepdims=True)
    v = jnp.var(x, axis=axis, keepdims=True)
    return (x - m) / jnp.sqrt(v + eps)
def _scatter_add(tgt, idx, src, axis=0):
    return tgt.at[idx].add(src)
def _segment_sum(src, seg, n):
    return jax.ops.segment_sum(src, seg, n)
class _Rng:
    def __init__(self, key):
        self._k = key
    def _next(self):
        self._k, sub = jax.random.split(self._k)
        return sub
    def normal(self, shape):
        return jax.random.normal(self._next(), shape, dtype=jnp.bfloat16)
    def randint(self, lo, hi, shape):
        return jax.random.randint(self._next(), shape, lo, hi, dtype=jnp.int32)
    def uniform(self, shape, lo=0.0, hi=1.0):
        return jax.random.uniform(self._next(), shape, jnp.bfloat16, lo, hi)
    def permutation(self, n):
        return jax.random.permutation(self._next(), n)


kernel_name = 'standalone__detection_seg_fpn_lateral__vision'

def setup_inputs():
    _rng = _Rng(jax.random.key(int.from_bytes(__import__("os").urandom(4), "little")))
    _w = (lambda a: (lambda t: t.astype(jnp.bfloat16) if jnp.issubdtype(t.dtype, jnp.floating) else t)(jnp.asarray(a)))
    H = W = (256 // 2) * 2
    C = 384
    k = 1
    return {
        "c_fine": _w((lambda *s: _rng.normal(s) * 0.05)(1, H, W, C)),
        "p_coarse": _w((lambda *s: _rng.normal(s) * 0.05)(1, H // 2, W // 2, C)),
        "w_lat": _w((lambda *s: _rng.normal(s) * 0.05)(C, C)),
        "w_out": _w((lambda *s: _rng.normal(s) * 0.05)(k, k, C, C)),
    }

def reference(c_fine, p_coarse, w_lat, w_out):
    B, H, W, C = c_fine.shape
    k = 1
    lat = jnp.einsum("bhwc,cd->bhwd", c_fine, w_lat)
    up = jnp.repeat(jnp.repeat(p_coarse, 2, axis=1), 2, axis=2)
    m = lat + up
    pad = k // 2
    mp = jnp.pad(m, ((0, 0), (pad, pad), (pad, pad), (0, 0)))
    o = None
    for di in range(k):
        for dj in range(k):
            t = jnp.einsum("bhwc,cd->bhwd", mp[:, di:di + H, dj:dj + W, :], w_out[di, dj])
            o = t if o is None else o + t
    return o
```

```python
import jax
import jax.numpy as jnp
import jax.experimental.pallas as pl
import jax.experimental.pallas.tpu as pltpu


def _dot(a, b):
    return jnp.dot(a, b, preferred_element_type=jnp.float32)


@jax.jit
def pallas_standalone__detection_seg_fpn_lateral__vision_kernel(
    c_fine: jax.Array,
    p_coarse: jax.Array,
    w_lat: jax.Array,
    w_out: jax.Array,
):
    read_ends, j0, A, r, first, per_it, tail_rows = (1, 2, 4, 7, 12, 19), 19, 8, 32, 64, 16, 512
    S, SPI = 1024, 2
    Bn, H, W, C = c_fine.shape
    dt = c_fine.dtype
    NS = Bn * H * W // S
    NI = NS // SPI
    rp = SPI * S // (2 * W)
    c2 = c_fine.reshape(NS, S, C)
    p2 = p_coarse.reshape(NS, S // 4, C)
    wo = w_out.reshape(C, C)
    J = S // r
    NW = NS // A * J
    ends = tuple(read_ends) + (NI,)
    cp_ = pltpu.make_async_copy

    def body(c_hbm, p_hbm, wl_hbm, wo_hbm, o_hbm, cb, pb, wl_ref, wo_ref, wc_ref, qs, sem):
        nseg = len(ends)
        W_SEM, T_SEM, O_SEM = nseg, nseg + 1, nseg + 2
        wcp = [cp_(wl_hbm, wl_ref, sem.at[W_SEM]), cp_(wo_hbm, wo_ref, sem.at[W_SEM])]
        for d in wcp:
            d.start()
        rds = []
        lo = 0
        for k, hi in enumerate(ends):
            sl = pl.ds(lo * SPI, (hi - lo) * SPI)
            ds = [cp_(p_hbm.at[sl], pb.at[sl], sem.at[k])]
            if k < nseg - 1:
                ds.append(cp_(c_hbm.at[sl], cb.at[sl], sem.at[k]))
            else:
                sl2 = pl.ds(lo * SPI, (hi - lo) * SPI - 1)
                ds.append(cp_(c_hbm.at[sl2], cb.at[sl2], sem.at[k]))
                i0 = (NS - 1, pl.ds(0, S - tail_rows))
                ds.append(cp_(c_hbm.at[i0], cb.at[i0], sem.at[k]))
            for d in ds:
                d.start()
            rds.append(ds)
            lo = hi
        it = (NS - 1, pl.ds(S - tail_rows, tail_rows))
        tail = cp_(c_hbm.at[it], cb.at[it], sem.at[T_SEM])
        tail.start()
        for d in wcp:
            d.wait()
        wc_ref[...] = _dot(wl_ref[...], wo_ref[...]).astype(dt)

        def write(t):
            idx = (pl.ds((t // J) * A, A), pl.ds(pl.multiple_of((t % J) * r, r), r))
            cp_(cb.at[idx], o_hbm.at[idx], sem.at[O_SEM]).start()

        def issued(i):
            avail = (i * SPI // A) * J
            return jnp.where(i < j0, 0, jnp.minimum(avail, first + per_it * (i - j0)))

        @pl.loop(0, NI)
        def _(i):
            lo = 0
            for k, hi in enumerate(ends):
                @pl.when(i == lo)
                def _():
                    for d in rds[k]:
                        d.wait()
                lo = hi

            @pl.loop(issued(i - 1), issued(i))
            def _(t):
                write(t)

            @pl.when(i == NI - 1)
            def _():
                tail.wait()

            sl = pl.ds(i * SPI, SPI)
            q = _dot(pb[sl].reshape(SPI * S // 4, C), wo_ref[...])
            n = SPI * S // 4
            for k in range(C // 128):
                qs[k, pl.ds(0, n, stride=2), :] = q[:, k * 128:(k + 1) * 128]
                qs[k, pl.ds(1, n, stride=2), :] = q[:, k * 128:(k + 1) * 128]
            up = jnp.concatenate([qs[k] for k in range(C // 128)], axis=1).reshape(rp, 1, W, C)
            lat = _dot(cb[sl].reshape(SPI * S, C), wc_ref[...]).reshape(rp, 2, W, C)
            cb[sl] = (lat + up).reshape(SPI, S, C).astype(dt)

        @pl.loop(issued(NI - 1), NW)
        def _(t):
            write(t)

        cp_(cb, o_hbm, sem.at[O_SEM]).wait()

    out = pl.pallas_call(
        body,
        in_specs=[pl.BlockSpec(memory_space=pl.ANY)] * 4,
        out_specs=pl.BlockSpec(memory_space=pl.ANY),
        out_shape=jax.ShapeDtypeStruct(c2.shape, dt),
        scratch_shapes=[pltpu.VMEM(c2.shape, dt), pltpu.VMEM(p2.shape, dt),
                        pltpu.VMEM((C, C), dt), pltpu.VMEM((C, C), dt), pltpu.VMEM((C, C), dt),
                        pltpu.VMEM((C // 128, SPI * S // 2, 128), jnp.float32),
                        pltpu.SemaphoreType.DMA((len(ends) + 3,))],
        compiler_params=pltpu.CompilerParams(vmem_limit_bytes=100 << 20),
    )(c2, p2, w_lat, wo)
    return out.reshape(c_fine.shape)
```

```python
import jax
import jax.numpy as jnp
import jax.experimental.pallas as pl
import jax.experimental.pallas.tpu as pltpu

_LANES = 128
_ROW_STRIDE = 8
_UNIT_ROWS = 4
_READ_CUTS = 16
_READS_PER_UNIT = 26
_READS_AT_START = 48
_READ_TAIL = 4
_WRITE_CUTS = 16
_WRITES_AT_SWITCH = 64
_WRITES_PER_UNIT = 16


def _dot(a, b):
    return jnp.dot(a, b, preferred_element_type=jnp.float32)


def _divmod(x, n):
    assert n & (n - 1) == 0
    return x >> (n.bit_length() - 1), x & (n - 1)


def _kernel(c_hbm, p_hbm, wl_hbm, wo_hbm, o_hbm,
            x_buf, o_buf, wl_buf, wo_buf, w_buf, up_buf, o_sem):
    n_slabs, _, n_coarse, channels = p_hbm.shape
    width = 2 * n_coarse
    n_fine = 2 * width
    fine_cut, coarse_cut = n_fine // _READ_CUTS, n_coarse // _READ_CUTS
    out_cut = n_fine // _WRITE_CUTS
    n_units = n_slabs * _ROW_STRIDE // _UNIT_ROWS
    n_reads = n_units * _READ_CUTS
    n_writes = n_units // 2 * _WRITE_CUTS
    n_issuing = (n_reads - _READS_AT_START) // _READS_PER_UNIT
    n_prologue = n_reads - n_issuing * _READS_PER_UNIT
    switch = n_issuing + 1
    assert n_issuing >= 1 and switch + 2 < n_units
    tail_rows = _READ_TAIL * fine_cut
    head_rows = n_coarse + n_fine - tail_rows

    def locate(unit):
        pair, half = _divmod(unit, 2)
        group, col = _divmod(pair, _ROW_STRIDE)
        return (2 * group + half) * _UNIT_ROWS, col

    def main(x_sems, w_sems):
        def start_read(t):
            unit, cut = _divmod(t, _READ_CUTS)
            slab, col = locate(unit)
            slabs = pl.ds(slab, _UNIT_ROWS)
            src = pl.ds(pl.multiple_of(cut * fine_cut, fine_cut), fine_cut)
            dst = pl.ds(pl.multiple_of(n_coarse + cut * fine_cut, fine_cut), fine_cut)
            sem = jnp.where(t >= n_reads - _READ_TAIL, n_units, unit)
            pltpu.make_async_copy(
                c_hbm.at[slabs, col, src], x_buf.at[slabs, col, dst], x_sems.at[sem]
            ).start(priority=1)
            rows = pl.ds(pl.multiple_of(cut * coarse_cut, coarse_cut), coarse_cut)
            pltpu.make_async_copy(
                p_hbm.at[slabs, col, rows], x_buf.at[slabs, col, rows], x_sems.at[unit]
            ).start(priority=0)

        def wait_rows(unit, start, size, sem):
            slab, col = locate(unit)
            buf = x_buf.at[pl.ds(slab, _UNIT_ROWS), col, pl.ds(start, size)]
            pltpu.make_async_copy(buf, buf, x_sems.at[sem]).wait()

        def wait_unit(unit):
            wait_rows(unit, 0, n_coarse + n_fine, unit)

        def start_write(t):
            pair, cut = _divmod(t, _WRITE_CUTS)
            slab, col = locate(2 * pair)
            idx = (pl.ds(slab, 2 * _UNIT_ROWS), col,
                   pl.ds(pl.multiple_of(cut * out_cut, out_cut), out_cut))
            pltpu.make_async_copy(o_buf.at[idx], o_hbm.at[idx], o_sem.at[0]).start()

        def writes_before(unit):
            ready = (unit >> 1) * _WRITE_CUTS
            paced = _WRITES_AT_SWITCH + _WRITES_PER_UNIT * (unit - switch)
            return jnp.where(unit < switch, 0, jnp.minimum(ready, paced))

        def compute(unit, first_read=None):
            slab, col = locate(unit)
            for r in range(_UNIT_ROWS):
                q = _dot(x_buf[slab + r, col, pl.ds(0, n_coarse)], wo_buf[...])
                for k in range(channels // _LANES):
                    for phase in range(2):
                        up_buf[k, pl.ds(r * width + phase, n_coarse, stride=2), :] = (
                            q[:, k * _LANES:(k + 1) * _LANES])
                up = jnp.concatenate(
                    [up_buf[k, pl.ds(r * width, width)]
                     for k in range(channels // _LANES)], axis=1)
                for y in range(2):
                    if first_read is not None:
                        slot, n_slots = 2 * r + y, 2 * _UNIT_ROWS
                        for k in range(slot * _READS_PER_UNIT // n_slots,
                                       (slot + 1) * _READS_PER_UNIT // n_slots):
                            start_read(first_read + k)
                    fine = x_buf[slab + r, col, pl.ds(n_coarse + y * width, width)]
                    o_buf[slab + r, col, pl.ds(y * width, width)] = (
                        _dot(fine, w_buf[...]) + up).astype(o_buf.dtype)

        weights = [pltpu.make_async_copy(wl_hbm, wl_buf, w_sems.at[0]),
                   pltpu.make_async_copy(wo_hbm.at[0, 0], wo_buf, w_sems.at[1])]
        for copy in weights:
            copy.start()
        pl.loop(0, _READS_AT_START)(start_read)
        for copy in weights:
            copy.wait()
        w_buf[...] = _dot(wl_buf[...], wo_buf[...]).astype(w_buf.dtype)
        pl.loop(_READS_AT_START, n_prologue)(start_read)

        @pl.loop(0, n_issuing)
        def _(unit):
            wait_unit(unit)
            compute(unit, n_prologue + unit * _READS_PER_UNIT)

        @pl.loop(n_issuing, n_units)
        def _(unit):
            @pl.when(unit < switch)
            def _():
                wait_unit(unit)

            @pl.when(unit == switch)
            def _():
                pl.loop(switch, n_units - 1)(wait_unit)
                wait_rows(n_units - 1, 0, head_rows, n_units - 1)

            pl.loop(writes_before(unit - 1), writes_before(unit))(start_write)

            @pl.when(unit == switch + 1)
            def _():
                wait_rows(n_units - 1, head_rows, tail_rows, n_units)

            compute(unit)

        pl.loop(writes_before(n_units - 1), n_writes)(start_write)

    pl.run_scoped(main, pltpu.SemaphoreType.DMA((n_units + 1,)),
                  pltpu.SemaphoreType.DMA((2,)))
    pltpu.make_async_copy(o_buf, o_hbm, o_sem.at[0]).wait()


@jax.jit
def pallas_standalone__detection_seg_fpn_lateral__vision_kernel(
    c_fine: jax.Array,
    p_coarse: jax.Array,
    w_lat: jax.Array,
    w_out: jax.Array,
):
    batch, height, width, channels = c_fine.shape
    dtype = c_fine.dtype
    n_rows = batch * height // 2
    assert p_coarse.shape == (batch, height // 2, width // 2, channels)
    assert n_rows % (2 * _UNIT_ROWS * _ROW_STRIDE) == 0
    assert width % (16 * _READ_CUTS) == 0 and channels % _LANES == 0
    lead = (n_rows // _ROW_STRIDE, _ROW_STRIDE)
    fine_shape = (*lead, 2 * width, channels)

    out = pl.pallas_call(
        _kernel,
        in_specs=[pl.BlockSpec(memory_space=pl.ANY)] * 4,
        out_specs=pl.BlockSpec(memory_space=pl.ANY),
        out_shape=jax.ShapeDtypeStruct(fine_shape, dtype),
        scratch_shapes=[
            pltpu.VMEM((*lead, width // 2 + 2 * width, channels), dtype),
            pltpu.VMEM(fine_shape, dtype),
            pltpu.VMEM((channels, channels), dtype),
            pltpu.VMEM((channels, channels), dtype),
            pltpu.VMEM((channels, channels), dtype),
            pltpu.VMEM((channels // _LANES, _UNIT_ROWS * width, _LANES), jnp.float32),
            pltpu.SemaphoreType.DMA((1,)),
        ],
        compiler_params=pltpu.CompilerParams(
            vmem_limit_bytes=120 * 1024 * 1024,
            disable_bounds_checks=True,
        ),
    )(
        c_fine.reshape(fine_shape),
        p_coarse.reshape(*lead, width // 2, channels),
        w_lat,
        w_out,
    )
    return out.reshape(c_fine.shape)
```

```python
import jax
import jax.numpy as jnp
import jax.experimental.pallas as pl
import jax.experimental.pallas.tpu as pltpu

_LANES = 128
_ROW_STRIDE = 8
_UNIT_ROWS = 4
_CUTS = 16
_READS_PER_UNIT = 26
_READS_AT_START = 48
_TAIL_CUTS = 2
_WRITES_AT_SWITCH = 64
_WRITES_PER_UNIT = 16


def _dot(a, b):
    return jnp.dot(a, b, preferred_element_type=jnp.float32)


def _divmod(x, n):
    assert n & (n - 1) == 0
    return x >> (n.bit_length() - 1), x & (n - 1)


def _kernel(c_hbm, p_hbm, wl_hbm, wo_hbm, o_hbm,
            x_buf, o_buf, wl_buf, wo_buf, w_buf, up_buf, o_sem):
    n_slabs, _, n_coarse, channels = p_hbm.shape
    width = 2 * n_coarse
    n_fine = 2 * width
    fine_cut, coarse_cut = n_fine // _CUTS, n_coarse // _CUTS
    n_units = n_slabs * _ROW_STRIDE // _UNIT_ROWS
    n_tiles = n_units // 2
    n_reads = n_units * _CUTS
    n_writes = n_tiles * _CUTS
    n_issuing = (n_reads - _READS_AT_START) // _READS_PER_UNIT
    n_prologue = n_reads - n_issuing * _READS_PER_UNIT
    switch = n_issuing + 1
    assert n_issuing >= 1 and switch + 2 < n_units
    tail = _TAIL_CUTS * fine_cut
    head = n_coarse + n_fine - tail

    def locate(tile, half=0):
        group, col = _divmod(tile, _ROW_STRIDE)
        return (2 * group + half) * _UNIT_ROWS, col

    def main(x_sems, w_sems):
        def start_read(t):
            tile, cut = _divmod(t >> 1, _CUTS)
            slab, col = locate(tile, t & 1)
            slabs = pl.ds(slab, _UNIT_ROWS)
            src = pl.ds(pl.multiple_of(cut * fine_cut, fine_cut), fine_cut)
            dst = pl.ds(pl.multiple_of(n_coarse + cut * fine_cut, fine_cut), fine_cut)
            sem = jnp.where(t >= n_reads - 2 * _TAIL_CUTS, n_tiles, tile)
            pltpu.make_async_copy(
                c_hbm.at[slabs, col, src], x_buf.at[slabs, col, dst], x_sems.at[sem]
            ).start(priority=1)
            rows = pl.ds(pl.multiple_of(cut * coarse_cut, coarse_cut), coarse_cut)
            pltpu.make_async_copy(
                p_hbm.at[slabs, col, rows], x_buf.at[slabs, col, rows], x_sems.at[tile]
            ).start(priority=0)

        def wait_part(tile, start, size, sem):
            slab, col = locate(tile)
            buf = x_buf.at[pl.ds(slab, 2 * _UNIT_ROWS), col, pl.ds(start, size)]
            pltpu.make_async_copy(buf, buf, x_sems.at[sem]).wait()

        def wait_tile(tile):
            wait_part(tile, 0, n_coarse + n_fine, tile)

        def wait_unit(unit):
            @pl.when((unit & 1) == 0)
            def _():
                wait_tile(unit >> 1)

        def start_write(t):
            tile, cut = _divmod(t, _CUTS)
            slab, col = locate(tile)
            idx = (pl.ds(slab, 2 * _UNIT_ROWS), col,
                   pl.ds(pl.multiple_of(cut * fine_cut, fine_cut), fine_cut))
            pltpu.make_async_copy(o_buf.at[idx], o_hbm.at[idx], o_sem.at[0]).start()

        def writes_before(unit):
            ready = (unit >> 1) * _CUTS
            paced = _WRITES_AT_SWITCH + _WRITES_PER_UNIT * (unit - switch)
            return jnp.where(unit < switch, 0, jnp.minimum(ready, paced))

        def compute(unit, first_read=None):
            slab, col = locate(unit >> 1, unit & 1)
            for r in range(_UNIT_ROWS):
                q = _dot(x_buf[slab + r, col, pl.ds(0, n_coarse)], wo_buf[...])
                for k in range(channels // _LANES):
                    for phase in range(2):
                        up_buf[k, pl.ds(r * width + phase, n_coarse, stride=2), :] = (
                            q[:, k * _LANES:(k + 1) * _LANES])
                up = jnp.concatenate(
                    [up_buf[k, pl.ds(r * width, width)]
                     for k in range(channels // _LANES)], axis=1)
                for y in range(2):
                    if first_read is not None:
                        slot, n_slots = 2 * r + y, 2 * _UNIT_ROWS
                        for k in range(slot * _READS_PER_UNIT // n_slots,
                                       (slot + 1) * _READS_PER_UNIT // n_slots):
                            start_read(first_read + k)
                    fine = x_buf[slab + r, col, pl.ds(n_coarse + y * width, width)]
                    o_buf[slab + r, col, pl.ds(y * width, width)] = (
                        _dot(fine, w_buf[...]) + up).astype(o_buf.dtype)

        weights = [pltpu.make_async_copy(wl_hbm, wl_buf, w_sems.at[0]),
                   pltpu.make_async_copy(wo_hbm.at[0, 0], wo_buf, w_sems.at[1])]
        for copy in weights:
            copy.start()
        pl.loop(0, _READS_AT_START)(start_read)
        for copy in weights:
            copy.wait()
        w_buf[...] = _dot(wl_buf[...], wo_buf[...]).astype(w_buf.dtype)
        pl.loop(_READS_AT_START, n_prologue)(start_read)

        @pl.loop(0, n_issuing)
        def _(unit):
            wait_unit(unit)
            compute(unit, n_prologue + unit * _READS_PER_UNIT)

        @pl.loop(n_issuing, n_units)
        def _(unit):
            @pl.when(unit < switch)
            def _():
                wait_unit(unit)

            @pl.when(unit == switch)
            def _():
                pl.loop((switch + 1) // 2, n_tiles - 1)(wait_tile)
                wait_part(n_tiles - 1, 0, head, n_tiles - 1)

            pl.loop(writes_before(unit - 1), writes_before(unit))(start_write)

            @pl.when(unit == switch + 1)
            def _():
                wait_part(n_tiles - 1, head, tail, n_tiles)

            compute(unit)

        pl.loop(writes_before(n_units - 1), n_writes)(start_write)

    pl.run_scoped(main, pltpu.SemaphoreType.DMA((n_tiles + 1,)),
                  pltpu.SemaphoreType.DMA((2,)))
    pltpu.make_async_copy(o_buf, o_hbm, o_sem.at[0]).wait()


@jax.jit
def pallas_standalone__detection_seg_fpn_lateral__vision_kernel(
    c_fine: jax.Array,
    p_coarse: jax.Array,
    w_lat: jax.Array,
    w_out: jax.Array,
):
    batch, height, width, channels = c_fine.shape
    dtype = c_fine.dtype
    n_rows = batch * height // 2
    assert p_coarse.shape == (batch, height // 2, width // 2, channels)
    assert n_rows % (2 * _UNIT_ROWS * _ROW_STRIDE) == 0
    assert width % (16 * _CUTS) == 0 and channels % _LANES == 0
    lead = (n_rows // _ROW_STRIDE, _ROW_STRIDE)
    fine_shape = (*lead, 2 * width, channels)

    out = pl.pallas_call(
        _kernel,
        in_specs=[pl.BlockSpec(memory_space=pl.ANY)] * 4,
        out_specs=pl.BlockSpec(memory_space=pl.ANY),
        out_shape=jax.ShapeDtypeStruct(fine_shape, dtype),
        scratch_shapes=[
            pltpu.VMEM((*lead, width // 2 + 2 * width, channels), dtype),
            pltpu.VMEM(fine_shape, dtype),
            pltpu.VMEM((channels, channels), dtype),
            pltpu.VMEM((channels, channels), dtype),
            pltpu.VMEM((channels, channels), dtype),
            pltpu.VMEM((channels // _LANES, _UNIT_ROWS * width, _LANES), jnp.float32),
            pltpu.SemaphoreType.DMA((1,)),
        ],
        compiler_params=pltpu.CompilerParams(vmem_limit_bytes=120 * 1024 * 1024),
    )(
        c_fine.reshape(fine_shape),
        p_coarse.reshape(*lead, width // 2, channels),
        w_lat,
        w_out,
    )
    return out.reshape(c_fine.shape)
```
